```python
import os as _os
_os.environ.setdefault("JAX_PLATFORMS", "cpu")
import jax
import jax.numpy as jnp

def _softmax(x, axis=-1):
    return jax.nn.softmax(x, axis=axis)
def _gelu(x):
    return jax.nn.gelu(x, approximate=True)
def _silu(x):
    return jax.nn.silu(x)
def _sigmoid(x):
    return jax.nn.sigmoid(x)
def _layernorm(x, axis=-1, eps=1e-5):
    m = jnp.mean(x, axis=axis, keepdims=True)
    v = jnp.var(x, axis=axis, keepdims=True)
    return (x - m) / jnp.sqrt(v + eps)
def _scatter_add(tgt, idx, src, axis=0):
    return tgt.at[idx].add(src)
def _segment_sum(src, seg, n):
    return jax.ops.segment_sum(src, seg, n)
class _Rng:
    def __init__(self, key):
        self._k = key
    def _next(self):
        self._k, sub = jax.random.split(self._k)
        return sub
    def normal(self, shape):
        return jax.random.normal(self._next(), shape, dtype=jnp.bfloat16)
    def randint(self, lo, hi, shape):
        return jax.random.randint(self._next(), shape, lo, hi, dtype=jnp.int32)
    def uniform(self, shape, lo=0.0, hi=1.0):
        return jax.random.uniform(self._next(), shape, jnp.bfloat16, lo, hi)
    def permutation(self, n):
        return jax.random.permutation(self._next(), n)


kernel_name = 'standalone__dense_activation_gelu__prompt'

def setup_inputs():
    _rng = _Rng(jax.random.key(int.from_bytes(__import__("os").urandom(4), "little")))
    _w = (lambda a: (lambda t: t.astype(jnp.bfloat16) if jnp.issubdtype(t.dtype, jnp.floating) else t)(jnp.asarray(a)))
    B, S, D, F = 1, 2048, 640, 1728
    return {
        "x": _w((lambda *s: _rng.normal(s) * 0.05)(B, S, D)),
        "w1": _w((lambda *s: _rng.normal(s) * 0.05)(D, F) * (D ** -0.5)),
        "b1": _w((lambda *s: _rng.normal(s) * 0.05)(F) * 0.01),
        "w2": _w((lambda *s: _rng.normal(s) * 0.05)(F, D) * (F ** -0.5)),
        "b2": _w((lambda *s: _rng.normal(s) * 0.05)(D) * 0.01),
    }

def reference(x, w1, b1, w2, b2):
    h = jnp.einsum("bsd,df->bsf", x, w1) + b1
    h = _gelu(h)
    return jnp.einsum("bsf,fd->bsd", h, w2) + b2
```

```python
import jax
import jax.numpy as jnp
from jax import lax
import jax.experimental.pallas as pl
import jax.experimental.pallas.tpu as pltpu
import functools

TM = 256
C1 = [128, 256, 512, 640, 192]
SPLIT0 = [2, 2, 1, 1, 2]
NIT = 2
SCOPES = False

import contextlib
def scope(n):
    return jax.named_scope(n) if SCOPES else contextlib.nullcontext()

def _gelu(h):
    c = 0.7978845608028654
    u = h * (c + (c * 0.044715) * (h * h))
    return 0.5 * h * (1.0 + jnp.tanh(u))

def _nt(a, b):
    return lax.dot_general(a, b, (((1,), (1,)), ((), ())), preferred_element_type=jnp.float32)

def _kernel(x_hbm, w1t_hbm, b1_hbm, w2_hbm, b2_hbm, o_hbm,
            xbuf, w1buf, b1buf, w2buf, b2buf, obuf, sems, osems):
    M, D = x_hbm.shape
    F = w1t_hbm.shape[0]
    nb = M // TM
    NT = D // 128
    assert sum(C1) == F
    bpi = (nb - 2) // NIT
    assert bpi * NIT == nb - 2
    nsem = [0]
    def mk(src, dst):
        s = sems.at[nsem[0]]
        nsem[0] += 1
        return pltpu.make_async_copy(src, dst, s)
    def rows(ref, r0, n): return ref.at[pl.ds(r0, n)]
    c1 = []
    f = 0
    for n in C1:
        c1.append((f, n)); f += n
    x0_cp = mk(rows(x_hbm, 0, TM), rows(xbuf, 0, TM))
    x1_cp = mk(rows(x_hbm, TM, TM), rows(xbuf, TM, TM))
    xr_cp = [mk(rows(x_hbm, (2 + i * bpi) * TM, bpi * TM), rows(xbuf, (2 + i * bpi) * TM, bpi * TM)) for i in range(NIT)]
    w1_cp = [mk(rows(w1t_hbm, f0, fs), rows(w1buf, f0, fs)) for f0, fs in c1]
    w2_cp = mk(w2_hbm, w2buf)
    b1_cp = mk(b1_hbm, b1buf)
    b2_cp = mk(b2_hbm, b2buf)

    b1_cp.start()
    x0_cp.start()
    for c in w1_cp[:-1]: c.start()
    x1_cp.start()
    w1_cp[-1].start()
    b2_cp.start()
    w2_cp.start()
    for c in xr_cp: c.start()

    def mm1(r0, b1, first=False):
        if not first:
            xb = xbuf[pl.ds(r0, TM), :]
            h = _nt(xb, w1buf[...]) + b1
            return [(0, F, [(0, TM, _gelu(h).astype(jnp.bfloat16))])]
        out = []
        for ci, (f0, fs) in enumerate(c1):
            with scope(f"w1_{ci}"):
                w1_cp[ci].wait()
                if ci == len(c1) - 1: x1_cp.wait()
            parts = []
            rs = TM // SPLIT0[ci]
            for s in range(SPLIT0[ci]):
                xb = xbuf[pl.ds(r0 + s * rs, rs), :]
                h = _nt(xb, w1buf[pl.ds(f0, fs), :]) + b1[:, f0:f0 + fs]
                parts.append((s * rs, rs, _gelu(h).astype(jnp.bfloat16)))
            out.append((f0, fs, parts))
        return out

    def assemble(gl):
        cols = []
        for f0, fs, parts in gl:
            cols.append(parts[0][2] if len(parts) == 1 else jnp.concatenate([p[2] for p in parts], axis=0))
        return cols[0] if len(cols) == 1 else jnp.concatenate(cols, axis=1)

    def ocopy(bi, r0, n=None):
        if n is None:
            return pltpu.make_async_copy(rows(obuf, r0, TM), rows(o_hbm, r0, TM), osems.at[bi * NT])
        cs = pl.ds(n * 128, 128)
        return pltpu.make_async_copy(obuf.at[pl.ds(r0, TM), cs], o_hbm.at[pl.ds(r0, TM), cs], osems.at[bi * NT + n])

    def mm2(bi, r0, g, b2, last=False):
        if not last:
            o = jnp.dot(g, w2buf[...], preferred_element_type=jnp.float32) + b2
            obuf[pl.ds(r0, TM), :] = o.astype(obuf.dtype)
            ocopy(bi, r0).start()
        else:
            for n in range(NT):
                cs = pl.ds(n * 128, 128)
                o = jnp.dot(g, w2buf[:, cs], preferred_element_type=jnp.float32) + b2[:, n * 128:(n + 1) * 128]
                obuf[pl.ds(r0, TM), cs] = o.astype(obuf.dtype)
                ocopy(bi, r0, n).start()

    with scope("w_x0"):
        b1_cp.wait()
        x0_cp.wait()
    b1 = b1buf[...].astype(jnp.float32)[None, :]
    g0 = assemble(mm1(0, b1, first=True))
    g1 = assemble(mm1(TM, b1))
    with scope("w_w2"):
        b2_cp.wait()
        w2_cp.wait()
    b2 = b2buf[...].astype(jnp.float32)[None, :]
    mm2(0, 0, g0, b2)
    mm2(1, TM, g1, b2)

    def body(it, carry):
        with scope("w_xr"):
            base = 2 + it * bpi
            r0 = pl.multiple_of(base * TM, TM)
            pltpu.make_async_copy(rows(x_hbm, r0, bpi * TM), rows(xbuf, r0, bpi * TM), sems.at[2 + it]).wait()
        b1 = b1buf[...].astype(jnp.float32)[None, :]
        b2 = b2buf[...].astype(jnp.float32)[None, :]
        for j in range(bpi):
            bi = base + j
            r = pl.multiple_of(bi * TM, TM)
            g = assemble(mm1(r, b1))
            mm2(bi, r, g, b2, last=(j == bpi - 1))
        return carry
    if NIT == 1:
        body(0, None)
    else:
        lax.fori_loop(0, NIT, body, None)
    with scope("w_out"):
        for bi in range(nb):
            if bi >= 2 and (bi - 2) % bpi == bpi - 1:
                for n in range(NT): ocopy(bi, bi * TM, n).wait()
            else:
                ocopy(bi, bi * TM).wait()

@jax.jit
def pallas_standalone__dense_activation_gelu__prompt_kernel(x, w1, b1, w2, b2):
    B, S, D = x.shape
    F = w1.shape[1]
    M = B * S
    x2 = x.reshape(M, D)
    hbm = pl.BlockSpec(memory_space=pltpu.MemorySpace.HBM)
    out = pl.pallas_call(
        _kernel,
        in_specs=[hbm] * 5,
        out_specs=hbm,
        out_shape=jax.ShapeDtypeStruct((M, D), x.dtype),
        scratch_shapes=[
            pltpu.VMEM((M, D), x.dtype),
            pltpu.VMEM((F, D), w1.dtype),
            pltpu.VMEM((F,), b1.dtype),
            pltpu.VMEM((F, D), w2.dtype),
            pltpu.VMEM((D,), b2.dtype),
            pltpu.VMEM((M, D), x.dtype),
            pltpu.SemaphoreType.DMA((16,)),
            pltpu.SemaphoreType.DMA(((M // TM) * (D // 128),)),
        ],
        compiler_params=pltpu.CompilerParams(
            vmem_limit_bytes=100 * 1024 * 1024,
        ),
    )(x2, w1.T, b1, w2, b2)
    return out.reshape(B, S, D)
```

```python
import jax
import jax.numpy as jnp
from jax import lax
import jax.experimental.pallas as pl
import jax.experimental.pallas.tpu as pltpu

_LANE = 128
_B0 = 512
_B1 = 384
_BLOCKS = (512, 512, 128)
_KGROUPS = (512, 512)
_CHUNKS = (512, 192)
_KORDER = ((0, 0), (0, 1), (1, 0), (1, 1), (2, 0), (2, 1), (3, 1), (4, 1), (3, 0), (4, 0))
_STAGE_A = 2


def _gelu(h):
    c = 0.7978845608028654
    u = h * (c + (c * 0.044715) * (h * h))
    return 0.5 * h * (1.0 + jnp.tanh(u))


def _nt(a, b):
    return lax.dot_general(a, b, (((1,), (1,)), ((), ())),
                           preferred_element_type=jnp.float32)


def _spans(sizes, start=0):
    out = []
    for n in sizes:
        out.append((start, n))
        start += n
    return out


def _mlp_kernel(x_hbm, w1t_hbm, b1_hbm, w2_hbm, b2_hbm, o_hbm,
                xbuf, w1buf, b1buf, w2buf, b2buf, obuf, hbuf, out_sem):
    M, D = x_hbm.shape
    F = w1t_hbm.shape[0]
    NT = D // _LANE
    FM = (F // _LANE) * _LANE
    groups = _spans(_KGROUPS)
    chunks = _spans(_CHUNKS, sum(_KGROUPS))
    blocks = _spans(_BLOCKS, _B0 + _B1)
    assert sum(_KGROUPS) + sum(_CHUNKS) == F and _B0 + _B1 + sum(_BLOCKS) == M
    cp = pltpu.make_async_copy
    f32 = jnp.float32
    dt = obuf.dtype

    def rows(ref, r0, n):
        return ref.at[pl.ds(r0, n)]

    def ktile(k):
        return pl.ds(k * _LANE, _LANE)

    def main(sems):
        nsem = 0
        issue, kcopies, seen = [], [], []
        for idx, (k, g) in enumerate(_KORDER):
            f0, fs = groups[g]
            sem = sems.at[nsem]
            nsem += 1
            piece = []
            if k not in seen:
                seen.append(k)
                piece.append(cp(x_hbm.at[pl.ds(0, _B0), ktile(k)],
                                xbuf.at[pl.ds(0, _B0), ktile(k)], sem))
            piece.append(cp(w1t_hbm.at[pl.ds(f0, fs), ktile(k)],
                            w1buf.at[pl.ds(f0, fs), ktile(k)], sem))
            kcopies.append(piece)
            issue += piece
            if idx == 3:
                bias_cps = [cp(b1_hbm, b1buf, sems.at[nsem]),
                            cp(b2_hbm, b2buf, sems.at[nsem])]
                nsem += 1
                issue += bias_cps
        chunk_cps = []
        for f0, fs in chunks:
            chunk_cps.append(cp(rows(w1t_hbm, f0, fs), rows(w1buf, f0, fs), sems.at[nsem]))
            nsem += 1
        x1_cp = cp(rows(x_hbm, _B0, _B1), rows(xbuf, _B0, _B1), sems.at[nsem])
        w2_cp = cp(w2_hbm, w2buf, sems.at[nsem + 1])
        nsem += 2
        block_cps = []
        for r0, tm in blocks:
            block_cps.append(cp(rows(x_hbm, r0, tm), rows(xbuf, r0, tm), sems.at[nsem]))
            nsem += 1
        issue += chunk_cps + [x1_cp, w2_cp] + block_cps
        for c in issue:
            c.start()

        def hidden(xb, b1, f0, fs):
            out = []
            tail = None
            if f0 + fs == F and FM < F:
                ht = _nt(w1buf[pl.ds(FM, F - FM), :], xb)
                tail = (FM, F - FM, _gelu(ht.T + b1[:, FM:]).astype(dt))
                fs = FM - f0
            if fs > 0:
                h = _nt(xb, w1buf[pl.ds(f0, fs), :]) + b1[:, f0:f0 + fs]
                out.append((f0, fs, _gelu(h).astype(dt)))
            if tail is not None:
                out.append(tail)
            return out

        def project(gs, cols):
            acc = None
            for f0, fs, g in gs:
                p = jnp.dot(g, w2buf[pl.ds(f0, fs), cols], preferred_element_type=f32)
                acc = p if acc is None else acc + p
            return acc

        def output(r0, tm, gs, b2, per_tile=False):
            if not per_tile:
                obuf[pl.ds(r0, tm), :] = (project(gs, slice(None)) + b2).astype(dt)
                cp(rows(obuf, r0, tm), rows(o_hbm, r0, tm), out_sem.at[0]).start()
                return
            for n in range(NT):
                o = project(gs, ktile(n)) + b2[:, n * _LANE:(n + 1) * _LANE]
                obuf[pl.ds(r0, tm), ktile(n)] = o.astype(dt)
                cp(obuf.at[pl.ds(r0, tm), ktile(n)],
                   o_hbm.at[pl.ds(r0, tm), ktile(n)], out_sem.at[0]).start()

        acc = [None] * len(groups)
        left = [NT] * len(groups)
        bias = []
        g0 = []

        def kstep(idx):
            k, g = _KORDER[idx]
            f0, fs = groups[g]
            for c in kcopies[idx]:
                c.wait()
            if idx == 4:
                for c in bias_cps:
                    c.wait()
                bias.append(b1buf[...].astype(f32)[None, :])
                bias.append(b2buf[...].astype(f32)[None, :])
            p = _nt(xbuf[pl.ds(0, _B0), ktile(k)], w1buf[pl.ds(f0, fs), ktile(k)])
            acc[g] = p if acc[g] is None else acc[g] + p
            left[g] -= 1
            if left[g] == 0:
                g0.append((f0, fs, _gelu(acc[g] + bias[0][:, f0:f0 + fs]).astype(dt)))

        for idx in range(_STAGE_A):
            kstep(idx)
        staged = [g for g in range(len(groups)) if acc[g] is not None]
        for g in staged:
            hbuf[:, pl.ds(*groups[g])] = acc[g]

        def rest(i):
            for g in staged:
                acc[g] = hbuf[:, pl.ds(*groups[g])]
            for idx in range(_STAGE_A, len(_KORDER)):
                kstep(idx)
            b1, b2 = bias
            gs0 = sorted(g0, key=lambda t: t[0])
            for c, (f0, fs) in zip(chunk_cps, chunks):
                c.wait()
                gs0 += hidden(xbuf[pl.ds(0, _B0), :], b1, f0, fs)
            x1_cp.wait()
            gs1 = hidden(xbuf[pl.ds(_B0, _B1), :], b1, 0, F)
            w2_cp.wait()
            output(0, _B0, gs0, b2)
            output(_B0, _B1, gs1, b2)
            for j, (c, (r0, tm)) in enumerate(zip(block_cps, blocks)):
                c.wait()
                gs = hidden(xbuf[pl.ds(r0, tm), :], b1, 0, F)
                output(r0, tm, gs, b2, per_tile=(j == len(blocks) - 1))
            return i + 1

        lax.while_loop(lambda i: i < 1, rest, jnp.int32(0))

    n_in_sems = len(_KORDER) + 1 + len(_CHUNKS) + 2 + len(_BLOCKS)
    pl.run_scoped(main, pltpu.SemaphoreType.DMA((n_in_sems,)))
    cp(obuf, o_hbm, out_sem.at[0]).wait()


@jax.jit
def pallas_standalone__dense_activation_gelu__prompt_kernel(
    x: jax.Array,
    w1: jax.Array,
    b1: jax.Array,
    w2: jax.Array,
    b2: jax.Array,
):
    B, S, D = x.shape
    F = w1.shape[1]
    M = B * S
    hbm = pl.BlockSpec(memory_space=pltpu.MemorySpace.HBM)
    out = pl.pallas_call(
        _mlp_kernel,
        in_specs=[hbm] * 5,
        out_specs=hbm,
        out_shape=jax.ShapeDtypeStruct((M, D), x.dtype),
        scratch_shapes=[
            pltpu.VMEM((M, D), x.dtype),
            pltpu.VMEM((F, D), w1.dtype),
            pltpu.VMEM((F,), b1.dtype),
            pltpu.VMEM((F, D), w2.dtype),
            pltpu.VMEM((D,), b2.dtype),
            pltpu.VMEM((M, D), x.dtype),
            pltpu.VMEM((_B0, sum(_KGROUPS)), jnp.float32),
            pltpu.SemaphoreType.DMA((1,)),
        ],
        compiler_params=pltpu.CompilerParams(
            vmem_limit_bytes=64 * 1024 * 1024,
            flags={"XLA_TPU_RESCHEDULE_DMA_DONES": True},
        ),
    )(x.reshape(M, D), w1.T, b1, w2, b2)
    return out.reshape(B, S, D)
```

```python
import jax
import jax.numpy as jnp
from jax import lax
import jax.experimental.pallas as pl
import jax.experimental.pallas.tpu as pltpu

_LANE = 128
_B0 = 512
_B1 = 512
_BLOCKS = (512, 384, 128)
_KGROUPS = (512, 512)
_CHUNKS = (512, 192)
_KORDER = ((0, 1, 0), (0, 1, 1), (1, 2, 0), (1, 2, 1),
           (2, 3, 0), (2, 3, 1), (3, 5, 0), (3, 5, 1))
_STAGE_A = 2


def _gelu(h):
    c = 0.7978845608028654
    u = h * (c + (c * 0.044715) * (h * h))
    return 0.5 * h * (1.0 + jnp.tanh(u))


def _nt(a, b):
    return lax.dot_general(a, b, (((1,), (1,)), ((), ())),
                           preferred_element_type=jnp.float32)


def _spans(sizes, start=0):
    out = []
    for n in sizes:
        out.append((start, n))
        start += n
    return out


def _mlp_kernel(x_hbm, w1t_hbm, b1_hbm, w2_hbm, b2_hbm, o_hbm,
                xbuf, w1buf, b1buf, w2buf, b2buf, obuf, hbuf, out_sem):
    M, D = x_hbm.shape
    F = w1t_hbm.shape[0]
    NT = D // _LANE
    FM = (F // _LANE) * _LANE
    groups = _spans(_KGROUPS)
    chunks = _spans(_CHUNKS, sum(_KGROUPS))
    blocks = _spans(_BLOCKS, _B0 + _B1)
    assert sum(_KGROUPS) + sum(_CHUNKS) == F and _B0 + _B1 + sum(_BLOCKS) == M
    cp = pltpu.make_async_copy
    f32 = jnp.float32
    dt = obuf.dtype

    def rows(ref, r0, n):
        return ref.at[pl.ds(r0, n)]

    def ktile(k0, k1=None):
        return pl.ds(k0 * _LANE, ((k0 + 1 if k1 is None else k1) - k0) * _LANE)

    def main(sems):
        nsem = 0
        issue, kcopies, x_cols = [], [], 0
        for idx, (k0, k1, g) in enumerate(_KORDER):
            f0, fs = groups[g]
            sem = sems.at[nsem]
            nsem += 1
            piece = []
            if k1 > x_cols:
                assert k0 == x_cols
                x_cols = k1
                piece.append(cp(x_hbm.at[pl.ds(0, _B0), ktile(k0, k1)],
                                xbuf.at[pl.ds(0, _B0), ktile(k0, k1)], sem))
            piece.append(cp(w1t_hbm.at[pl.ds(f0, fs), ktile(k0, k1)],
                            w1buf.at[pl.ds(f0, fs), ktile(k0, k1)], sem))
            kcopies.append(piece)
            issue += piece
            if idx == 3:
                bias_cps = [cp(b1_hbm, b1buf, sems.at[nsem]),
                            cp(b2_hbm, b2buf, sems.at[nsem])]
                nsem += 1
                issue += bias_cps
        chunk_cps = []
        for f0, fs in chunks:
            chunk_cps.append(cp(rows(w1t_hbm, f0, fs), rows(w1buf, f0, fs), sems.at[nsem]))
            nsem += 1
        x1_cp = cp(rows(x_hbm, _B0, _B1), rows(xbuf, _B0, _B1), sems.at[nsem])
        w2_cp = cp(w2_hbm, w2buf, sems.at[nsem + 1])
        nsem += 2
        block_cps = []
        for r0, tm in blocks:
            block_cps.append(cp(rows(x_hbm, r0, tm), rows(xbuf, r0, tm), sems.at[nsem]))
            nsem += 1
        issue += chunk_cps + [x1_cp, w2_cp] + block_cps
        for c in issue:
            c.start()

        def hidden(xb, b1, f0, fs):
            out = []
            tail = None
            if f0 + fs == F and FM < F:
                ht = _nt(w1buf[pl.ds(FM, F - FM), :], xb)
                tail = (FM, F - FM, _gelu(ht.T + b1[:, FM:]).astype(dt))
                fs = FM - f0
            if fs > 0:
                h = _nt(xb, w1buf[pl.ds(f0, fs), :]) + b1[:, f0:f0 + fs]
                out.append((f0, fs, _gelu(h).astype(dt)))
            if tail is not None:
                out.append(tail)
            return out

        def project(gs, cols):
            acc = None
            for f0, fs, g in gs:
                p = jnp.dot(g, w2buf[pl.ds(f0, fs), cols], preferred_element_type=f32)
                acc = p if acc is None else acc + p
            return acc

        def output(r0, tm, gs, b2, per_tile=False):
            if not per_tile:
                obuf[pl.ds(r0, tm), :] = (project(gs, slice(None)) + b2).astype(dt)
                cp(rows(obuf, r0, tm), rows(o_hbm, r0, tm), out_sem.at[0]).start()
                return
            for n in range(NT):
                o = project(gs, ktile(n)) + b2[:, n * _LANE:(n + 1) * _LANE]
                obuf[pl.ds(r0, tm), ktile(n)] = o.astype(dt)
                cp(obuf.at[pl.ds(r0, tm), ktile(n)],
                   o_hbm.at[pl.ds(r0, tm), ktile(n)], out_sem.at[0]).start()

        acc = [None] * len(groups)
        left = [NT] * len(groups)
        bias = []
        g0 = []

        def kstep(idx):
            k0, k1, g = _KORDER[idx]
            f0, fs = groups[g]
            for c in kcopies[idx]:
                c.wait()
            if idx == 4:
                for c in bias_cps:
                    c.wait()
                bias.append(b1buf[...].astype(f32)[None, :])
                bias.append(b2buf[...].astype(f32)[None, :])
            p = _nt(xbuf[pl.ds(0, _B0), ktile(k0, k1)], w1buf[pl.ds(f0, fs), ktile(k0, k1)])
            acc[g] = p if acc[g] is None else acc[g] + p
            left[g] -= k1 - k0
            if left[g] == 0:
                g0.append((f0, fs, _gelu(acc[g] + bias[0][:, f0:f0 + fs]).astype(dt)))

        for idx in range(_STAGE_A):
            kstep(idx)
        staged = [g for g in range(len(groups)) if acc[g] is not None]
        for g in staged:
            hbuf[:, pl.ds(*groups[g])] = acc[g]

        def rest(i):
            for g in staged:
                acc[g] = hbuf[:, pl.ds(*groups[g])]
            for idx in range(_STAGE_A, len(_KORDER)):
                kstep(idx)
            b1, b2 = bias
            gs0 = sorted(g0, key=lambda t: t[0])
            for c, (f0, fs) in zip(chunk_cps, chunks):
                c.wait()
                gs0 += hidden(xbuf[pl.ds(0, _B0), :], b1, f0, fs)
            x1_cp.wait()
            gs1 = hidden(xbuf[pl.ds(_B0, _B1), :], b1, 0, F)
            w2_cp.wait()
            output(0, _B0, gs0, b2)
            output(_B0, _B1, gs1, b2)
            for j, (c, (r0, tm)) in enumerate(zip(block_cps, blocks)):
                c.wait()
                gs = hidden(xbuf[pl.ds(r0, tm), :], b1, 0, F)
                output(r0, tm, gs, b2, per_tile=(j == len(blocks) - 1))
            return i + 1

        lax.while_loop(lambda i: i < 1, rest, jnp.int32(0))

    n_in_sems = len(_KORDER) + 1 + len(_CHUNKS) + 2 + len(_BLOCKS)
    pl.run_scoped(main, pltpu.SemaphoreType.DMA((n_in_sems,)))
    cp(obuf, o_hbm, out_sem.at[0]).wait()


@jax.jit
def pallas_standalone__dense_activation_gelu__prompt_kernel(
    x: jax.Array,
    w1: jax.Array,
    b1: jax.Array,
    w2: jax.Array,
    b2: jax.Array,
):
    B, S, D = x.shape
    F = w1.shape[1]
    M = B * S
    hbm = pl.BlockSpec(memory_space=pltpu.MemorySpace.HBM)
    out = pl.pallas_call(
        _mlp_kernel,
        in_specs=[hbm] * 5,
        out_specs=hbm,
        out_shape=jax.ShapeDtypeStruct((M, D), x.dtype),
        scratch_shapes=[
            pltpu.VMEM((M, D), x.dtype),
            pltpu.VMEM((F, D), w1.dtype),
            pltpu.VMEM((F,), b1.dtype),
            pltpu.VMEM((F, D), w2.dtype),
            pltpu.VMEM((D,), b2.dtype),
            pltpu.VMEM((M, D), x.dtype),
            pltpu.VMEM((_B0, sum(_KGROUPS)), jnp.float32),
            pltpu.SemaphoreType.DMA((1,)),
        ],
        compiler_params=pltpu.CompilerParams(
            vmem_limit_bytes=64 * 1024 * 1024,
            flags={"XLA_TPU_RESCHEDULE_DMA_DONES": True},
        ),
    )(x.reshape(M, D), w1.T, b1, w2, b2)
    return out.reshape(B, S, D)
```

```python
import jax
import jax.numpy as jnp
from jax import lax
import jax.experimental.pallas as pl
import jax.experimental.pallas.tpu as pltpu

_LANE = 128
_B0 = 512
_B1 = 512
_BLOCKS = (512, 384, 128)
_KGROUPS = (512, 512, 512)
_CHUNKS = (192,)
_KORDER = ((0, 1, 0), (0, 1, 1), (0, 1, 2),
           (1, 3, 0), (1, 3, 1), (1, 3, 2),
           (3, 5, 0), (3, 5, 1), (3, 5, 2))
_STAGE_A = 3


def _gelu(h):
    c = 0.7978845608028654
    u = h * (c + (c * 0.044715) * (h * h))
    return 0.5 * h * (1.0 + jnp.tanh(u))


def _nt(a, b):
    return lax.dot_general(a, b, (((1,), (1,)), ((), ())),
                           preferred_element_type=jnp.float32)


def _spans(sizes, start=0):
    out = []
    for n in sizes:
        out.append((start, n))
        start += n
    return out


def _mlp_kernel(x_hbm, w1t_hbm, b1_hbm, w2_hbm, b2_hbm, o_hbm,
                xbuf, w1buf, b1buf, w2buf, b2buf, obuf, hbuf, out_sem):
    M, D = x_hbm.shape
    F = w1t_hbm.shape[0]
    NT = D // _LANE
    FM = (F // _LANE) * _LANE
    groups = _spans(_KGROUPS)
    chunks = _spans(_CHUNKS, sum(_KGROUPS))
    blocks = _spans(_BLOCKS, _B0 + _B1)
    assert sum(_KGROUPS) + sum(_CHUNKS) == F and _B0 + _B1 + sum(_BLOCKS) == M
    cp = pltpu.make_async_copy
    f32 = jnp.float32
    dt = obuf.dtype

    def rows(ref, r0, n):
        return ref.at[pl.ds(r0, n)]

    def ktile(k0, k1=None):
        return pl.ds(k0 * _LANE, ((k0 + 1 if k1 is None else k1) - k0) * _LANE)

    def main(sems):
        nsem = 0
        issue, kcopies, x_cols = [], [], 0
        for idx, (k0, k1, g) in enumerate(_KORDER):
            f0, fs = groups[g]
            sem = sems.at[nsem]
            nsem += 1
            piece = []
            if k1 > x_cols:
                assert k0 == x_cols
                x_cols = k1
                piece.append(cp(x_hbm.at[pl.ds(0, _B0), ktile(k0, k1)],
                                xbuf.at[pl.ds(0, _B0), ktile(k0, k1)], sem))
            piece.append(cp(w1t_hbm.at[pl.ds(f0, fs), ktile(k0, k1)],
                            w1buf.at[pl.ds(f0, fs), ktile(k0, k1)], sem))
            kcopies.append(piece)
            issue += piece
            if idx == 3:
                bias_cps = [cp(b1_hbm, b1buf, sems.at[nsem]),
                            cp(b2_hbm, b2buf, sems.at[nsem])]
                nsem += 1
                issue += bias_cps
        chunk_cps = []
        for f0, fs in chunks:
            chunk_cps.append(cp(rows(w1t_hbm, f0, fs), rows(w1buf, f0, fs), sems.at[nsem]))
            nsem += 1
        x1_cp = cp(rows(x_hbm, _B0, _B1), rows(xbuf, _B0, _B1), sems.at[nsem])
        w2_cp = cp(w2_hbm, w2buf, sems.at[nsem + 1])
        nsem += 2
        block_cps = []
        for r0, tm in blocks:
            block_cps.append(cp(rows(x_hbm, r0, tm), rows(xbuf, r0, tm), sems.at[nsem]))
            nsem += 1
        issue += chunk_cps + [x1_cp, w2_cp] + block_cps
        for c in issue:
            c.start()

        def hidden(xb, b1, f0, fs):
            out = []
            tail = None
            if f0 + fs == F and FM < F:
                ht = _nt(w1buf[pl.ds(FM, F - FM), :], xb)
                tail = (FM, F - FM, _gelu(ht.T + b1[:, FM:]).astype(dt))
                fs = FM - f0
            if fs > 0:
                h = _nt(xb, w1buf[pl.ds(f0, fs), :]) + b1[:, f0:f0 + fs]
                out.append((f0, fs, _gelu(h).astype(dt)))
            if tail is not None:
                out.append(tail)
            return out

        def project(gs, cols):
            acc = None
            for f0, fs, g in gs:
                p = jnp.dot(g, w2buf[pl.ds(f0, fs), cols], preferred_element_type=f32)
                acc = p if acc is None else acc + p
            return acc

        def output(r0, tm, gs, b2, per_tile=False):
            if not per_tile:
                obuf[pl.ds(r0, tm), :] = (project(gs, slice(None)) + b2).astype(dt)
                cp(rows(obuf, r0, tm), rows(o_hbm, r0, tm), out_sem.at[0]).start()
                return
            for n in range(NT):
                o = project(gs, ktile(n)) + b2[:, n * _LANE:(n + 1) * _LANE]
                obuf[pl.ds(r0, tm), ktile(n)] = o.astype(dt)
                cp(obuf.at[pl.ds(r0, tm), ktile(n)],
                   o_hbm.at[pl.ds(r0, tm), ktile(n)], out_sem.at[0]).start()

        acc = [None] * len(groups)
        left = [NT] * len(groups)
        bias = []
        g0 = []

        def kstep(idx):
            k0, k1, g = _KORDER[idx]
            f0, fs = groups[g]
            for c in kcopies[idx]:
                c.wait()
            if idx == 4:
                for c in bias_cps:
                    c.wait()
                bias.append(b1buf[...].astype(f32)[None, :])
                bias.append(b2buf[...].astype(f32)[None, :])
            p = _nt(xbuf[pl.ds(0, _B0), ktile(k0, k1)], w1buf[pl.ds(f0, fs), ktile(k0, k1)])
            acc[g] = p if acc[g] is None else acc[g] + p
            left[g] -= k1 - k0
            if left[g] == 0:
                g0.append((f0, fs, _gelu(acc[g] + bias[0][:, f0:f0 + fs]).astype(dt)))

        for idx in range(_STAGE_A):
            kstep(idx)
        staged = [g for g in range(len(groups)) if acc[g] is not None]
        for g in staged:
            hbuf[:, pl.ds(*groups[g])] = acc[g]

        def rest(i):
            for g in staged:
                acc[g] = hbuf[:, pl.ds(*groups[g])]
            for idx in range(_STAGE_A, len(_KORDER)):
                kstep(idx)
            b1, b2 = bias
            gs0 = sorted(g0, key=lambda t: t[0])
            for c, (f0, fs) in zip(chunk_cps, chunks):
                c.wait()
                gs0 += hidden(xbuf[pl.ds(0, _B0), :], b1, f0, fs)
            x1_cp.wait()
            gs1 = hidden(xbuf[pl.ds(_B0, _B1), :], b1, 0, F)
            w2_cp.wait()
            output(0, _B0, gs0, b2)
            output(_B0, _B1, gs1, b2)
            for j, (c, (r0, tm)) in enumerate(zip(block_cps, blocks)):
                c.wait()
                gs = hidden(xbuf[pl.ds(r0, tm), :], b1, 0, F)
                output(r0, tm, gs, b2, per_tile=(j == len(blocks) - 1))
            return i + 1

        lax.while_loop(lambda i: i < 1, rest, jnp.int32(0))

    n_in_sems = len(_KORDER) + 1 + len(_CHUNKS) + 2 + len(_BLOCKS)
    pl.run_scoped(main, pltpu.SemaphoreType.DMA((n_in_sems,)))
    cp(obuf, o_hbm, out_sem.at[0]).wait()


@jax.jit
def pallas_standalone__dense_activation_gelu__prompt_kernel(
    x: jax.Array,
    w1: jax.Array,
    b1: jax.Array,
    w2: jax.Array,
    b2: jax.Array,
):
    B, S, D = x.shape
    F = w1.shape[1]
    M = B * S
    hbm = pl.BlockSpec(memory_space=pltpu.MemorySpace.HBM)
    out = pl.pallas_call(
        _mlp_kernel,
        in_specs=[hbm] * 5,
        out_specs=hbm,
        out_shape=jax.ShapeDtypeStruct((M, D), x.dtype),
        scratch_shapes=[
            pltpu.VMEM((M, D), x.dtype),
            pltpu.VMEM((F, D), w1.dtype),
            pltpu.VMEM((F,), b1.dtype),
            pltpu.VMEM((F, D), w2.dtype),
            pltpu.VMEM((D,), b2.dtype),
            pltpu.VMEM((M, D), x.dtype),
            pltpu.VMEM((_B0, sum(_KGROUPS)), jnp.float32),
            pltpu.SemaphoreType.DMA((1,)),
        ],
        compiler_params=pltpu.CompilerParams(
            vmem_limit_bytes=64 * 1024 * 1024,
            flags={"XLA_TPU_RESCHEDULE_DMA_DONES": True},
        ),
    )(x.reshape(M, D), w1.T, b1, w2, b2)
    return out.reshape(B, S, D)
```

```python
import jax
import jax.numpy as jnp
from jax import lax
import jax.experimental.pallas as pl
import jax.experimental.pallas.tpu as pltpu

_LANE = 128
_B0 = 512
_B1 = 512
_BLOCKS = (512, 384, 128)
_KGROUPS = (512, 512, 512)
_CHUNKS = (192,)
_KORDER = ((0, 1, 0), (0, 1, 1), (0, 1, 2),
           (1, 3, 0), (1, 3, 1), (1, 3, 2),
           (3, 5, 0), (3, 5, 1), (3, 5, 2))
_STAGES = (1, 3)
_BIAS_STEP = 4


def _gelu(h):
    c = 0.7978845608028654
    u = h * (c + (c * 0.044715) * (h * h))
    return 0.5 * h * (1.0 + jnp.tanh(u))


def _nt(a, b):
    return lax.dot_general(a, b, (((1,), (1,)), ((), ())),
                           preferred_element_type=jnp.float32)


def _spans(sizes, start=0):
    out = []
    for n in sizes:
        out.append((start, n))
        start += n
    return out


def _region(fn):
    def body(i):
        fn()
        return i + 1
    lax.while_loop(lambda i: i < 1, body, jnp.int32(0))


def _mlp_kernel(x_hbm, w1t_hbm, b1_hbm, w2_hbm, b2_hbm, o_hbm,
                xbuf, w1buf, b1buf, w2buf, b2buf, obuf, hbuf, out_sem):
    M, D = x_hbm.shape
    F = w1t_hbm.shape[0]
    NT = D // _LANE
    FM = (F // _LANE) * _LANE
    groups = _spans(_KGROUPS)
    chunks = _spans(_CHUNKS, sum(_KGROUPS))
    blocks = _spans(_BLOCKS, _B0 + _B1)
    assert sum(_KGROUPS) + sum(_CHUNKS) == F and _B0 + _B1 + sum(_BLOCKS) == M
    cp = pltpu.make_async_copy
    f32 = jnp.float32
    dt = obuf.dtype

    def rows(ref, r0, n):
        return ref.at[pl.ds(r0, n)]

    def ktile(k0, k1=None):
        return pl.ds(k0 * _LANE, ((k0 + 1 if k1 is None else k1) - k0) * _LANE)

    def main(sems):
        nsem = 0
        issue, kcopies, x_cols = [], [], 0
        for idx, (k0, k1, g) in enumerate(_KORDER):
            if idx == _BIAS_STEP:
                bias_cps = [cp(b1_hbm, b1buf, sems.at[nsem]),
                            cp(b2_hbm, b2buf, sems.at[nsem])]
                nsem += 1
                issue += bias_cps
            f0, fs = groups[g]
            sem = sems.at[nsem]
            nsem += 1
            piece = []
            if k1 > x_cols:
                assert k0 == x_cols
                x_cols = k1
                piece.append(cp(x_hbm.at[pl.ds(0, _B0), ktile(k0, k1)],
                                xbuf.at[pl.ds(0, _B0), ktile(k0, k1)], sem))
            piece.append(cp(w1t_hbm.at[pl.ds(f0, fs), ktile(k0, k1)],
                            w1buf.at[pl.ds(f0, fs), ktile(k0, k1)], sem))
            kcopies.append(piece)
            issue += piece
        chunk_cps = []
        for f0, fs in chunks:
            chunk_cps.append(cp(rows(w1t_hbm, f0, fs), rows(w1buf, f0, fs), sems.at[nsem]))
            nsem += 1
        x1_cp = cp(rows(x_hbm, _B0, _B1), rows(xbuf, _B0, _B1), sems.at[nsem])
        w2_cp = cp(w2_hbm, w2buf, sems.at[nsem + 1])
        nsem += 2
        block_cps = []
        for r0, tm in blocks:
            block_cps.append(cp(rows(x_hbm, r0, tm), rows(xbuf, r0, tm), sems.at[nsem]))
            nsem += 1
        issue += chunk_cps + [x1_cp, w2_cp] + block_cps
        for c in issue:
            c.start()

        def hidden(xb, b1, f0, fs):
            out = []
            tail = None
            if f0 + fs == F and FM < F:
                ht = _nt(w1buf[pl.ds(FM, F - FM), :], xb)
                tail = (FM, F - FM, _gelu(ht.T + b1[:, FM:]).astype(dt))
                fs = FM - f0
            if fs > 0:
                h = _nt(xb, w1buf[pl.ds(f0, fs), :]) + b1[:, f0:f0 + fs]
                out.append((f0, fs, _gelu(h).astype(dt)))
            if tail is not None:
                out.append(tail)
            return out

        def project(gs, cols):
            acc = None
            for f0, fs, g in gs:
                p = jnp.dot(g, w2buf[pl.ds(f0, fs), cols], preferred_element_type=f32)
                acc = p if acc is None else acc + p
            return acc

        def output(r0, tm, gs, b2, per_tile=False):
            if not per_tile:
                obuf[pl.ds(r0, tm), :] = (project(gs, slice(None)) + b2).astype(dt)
                cp(rows(obuf, r0, tm), rows(o_hbm, r0, tm), out_sem.at[0]).start()
                return
            for n in range(NT):
                o = project(gs, ktile(n)) + b2[:, n * _LANE:(n + 1) * _LANE]
                obuf[pl.ds(r0, tm), ktile(n)] = o.astype(dt)
                cp(obuf.at[pl.ds(r0, tm), ktile(n)],
                   o_hbm.at[pl.ds(r0, tm), ktile(n)], out_sem.at[0]).start()

        acc = [None] * len(groups)
        parked = [False] * len(groups)
        left = [NT] * len(groups)
        bias = []
        g0 = []

        def kstep(idx):
            k0, k1, g = _KORDER[idx]
            f0, fs = groups[g]
            for c in kcopies[idx]:
                c.wait()
            if idx == _BIAS_STEP:
                for c in bias_cps:
                    c.wait()
                bias.append(b1buf[...].astype(f32)[None, :])
                bias.append(b2buf[...].astype(f32)[None, :])
            p = _nt(xbuf[pl.ds(0, _B0), ktile(k0, k1)], w1buf[pl.ds(f0, fs), ktile(k0, k1)])
            if parked[g]:
                p = p + hbuf[:, pl.ds(f0, fs)]
                parked[g] = False
            acc[g] = p if acc[g] is None else acc[g] + p
            left[g] -= k1 - k0
            if left[g] == 0:
                g0.append((f0, fs, _gelu(acc[g] + bias[0][:, f0:f0 + fs]).astype(dt)))

        def stage(s):
            if s == len(_STAGES):
                return rest()
            for idx in range(_STAGES[s - 1] if s else 0, _STAGES[s]):
                kstep(idx)
            for g in range(len(groups)):
                if acc[g] is not None:
                    hbuf[:, pl.ds(*groups[g])] = acc[g]
                    acc[g], parked[g] = None, True
            _region(lambda: stage(s + 1))

        def rest():
            for idx in range(_STAGES[-1], len(_KORDER)):
                kstep(idx)
            b1, b2 = bias
            gs0 = sorted(g0, key=lambda t: t[0])
            for c, (f0, fs) in zip(chunk_cps, chunks):
                c.wait()
                gs0 += hidden(xbuf[pl.ds(0, _B0), :], b1, f0, fs)
            x1_cp.wait()
            gs1 = hidden(xbuf[pl.ds(_B0, _B1), :], b1, 0, F)
            w2_cp.wait()
            output(0, _B0, gs0, b2)
            output(_B0, _B1, gs1, b2)
            for j, (c, (r0, tm)) in enumerate(zip(block_cps, blocks)):
                c.wait()
                gs = hidden(xbuf[pl.ds(r0, tm), :], b1, 0, F)
                output(r0, tm, gs, b2, per_tile=(j == len(blocks) - 1))

        stage(0)

    n_in_sems = len(_KORDER) + 1 + len(_CHUNKS) + 2 + len(_BLOCKS)
    pl.run_scoped(main, pltpu.SemaphoreType.DMA((n_in_sems,)))
    cp(obuf, o_hbm, out_sem.at[0]).wait()


@jax.jit
def pallas_standalone__dense_activation_gelu__prompt_kernel(
    x: jax.Array,
    w1: jax.Array,
    b1: jax.Array,
    w2: jax.Array,
    b2: jax.Array,
):
    B, S, D = x.shape
    F = w1.shape[1]
    M = B * S
    hbm = pl.BlockSpec(memory_space=pltpu.MemorySpace.HBM)
    out = pl.pallas_call(
        _mlp_kernel,
        in_specs=[hbm] * 5,
        out_specs=hbm,
        out_shape=jax.ShapeDtypeStruct((M, D), x.dtype),
        scratch_shapes=[
            pltpu.VMEM((M, D), x.dtype),
            pltpu.VMEM((F, D), w1.dtype),
            pltpu.VMEM((F,), b1.dtype),
            pltpu.VMEM((F, D), w2.dtype),
            pltpu.VMEM((D,), b2.dtype),
            pltpu.VMEM((M, D), x.dtype),
            pltpu.VMEM((_B0, sum(_KGROUPS)), jnp.float32),
            pltpu.SemaphoreType.DMA((1,)),
        ],
        compiler_params=pltpu.CompilerParams(
            vmem_limit_bytes=64 * 1024 * 1024,
            flags={"XLA_TPU_RESCHEDULE_DMA_DONES": True},
        ),
    )(x.reshape(M, D), w1.T, b1, w2, b2)
    return out.reshape(B, S, D)
```
